```python
import os as _os
_os.environ.setdefault('JAX_PLATFORMS', 'cpu')
import jax
import jax.numpy as jnp

def _softmax(x, axis=-1):
    return jax.nn.softmax(x, axis=axis)

def _gelu(x):
    return jax.nn.gelu(x, approximate=True)

def _silu(x):
    return jax.nn.silu(x)

def _sigmoid(x):
    return jax.nn.sigmoid(x)

def _layernorm(x, axis=-1, eps=1e-05):
    m = jnp.mean(x, axis=axis, keepdims=True)
    v = jnp.var(x, axis=axis, keepdims=True)
    return (x - m) / jnp.sqrt(v + eps)

def _scatter_add(tgt, idx, src, axis=0):
    return tgt.at[idx].add(src)

def _segment_sum(src, seg, n):
    return jax.ops.segment_sum(src, seg, n)

class _Rng:

    def __init__(self, key):
        self._k = key

    def _next(self):
        self._k, sub = jax.random.split(self._k)
        return sub

    def normal(self, shape):
        return jax.random.normal(self._next(), shape, dtype=jnp.bfloat16)

    def randint(self, lo, hi, shape):
        return jax.random.randint(self._next(), shape, lo, hi, dtype=jnp.int32)

    def uniform(self, shape, lo=0.0, hi=1.0):
        return jax.random.uniform(self._next(), shape, jnp.bfloat16, lo, hi)

    def permutation(self, n):
        return jax.random.permutation(self._next(), n)
kernel_name = 'adaLN_cond__sliding_local_dilated__dense_activation_silu__prompt'

def setup_inputs():
    _rng = _Rng(jax.random.key(int.from_bytes(__import__("os").urandom(4), "little")))
    _w = lambda a: (lambda t: t.astype(jnp.bfloat16) if jnp.issubdtype(t.dtype, jnp.floating) else t)(jnp.asarray(a))

    def _A_setup():
        B, S, D = (1, 2048, 512)
        return {'x': _w((lambda *s: _rng.normal(s) * 0.05)(B, S, D)), 'wqkv': _w((lambda *s: _rng.normal(s) * 0.05)(D, 3 * D)), 'wo': _w((lambda *s: _rng.normal(s) * 0.05)(D, D))}
    _A_in = _A_setup()

    def _B_setup():
        B, S, D, F = (1, 2048, 512, 1792)
        return {'x': _w((lambda *s: _rng.normal(s) * 0.05)(B, S, D)), 'w1': _w((lambda *s: _rng.normal(s) * 0.8)(D, F) * D ** (-0.5)), 'w2': _w((lambda *s: _rng.normal(s) * 0.8)(F, D) * F ** (-0.5))}
    _B_in = _B_setup()
    return {'A_x': _A_in['x'], 'A_wqkv': _A_in['wqkv'], 'A_wo': _A_in['wo'], 'B_x': _B_in['x'], 'B_w1': _B_in['w1'], 'B_w2': _B_in['w2'], 'c': _w((lambda *s: _rng.normal(s) * 0.05)(1, 512) * 8.0), 'w_mod': _w((lambda *s: _rng.normal(s) * 0.05)(512, 6 * 512) * 512 ** (-0.5) * 8.0)}

def reference(A_x, A_wqkv, A_wo, B_x, B_w1, B_w2, c, w_mod):

    def _A_ref(x, wqkv, wo):
        B, S, D = x.shape
        H = 32
        Dh = D // H
        W, dil = (8, 2)
        qkv = (lambda x, *d: x.transpose(*d))((x @ wqkv).reshape(B, S, 3, H, Dh), 2, 0, 3, 1, 4)
        q, k, v = (qkv[0], qkv[1], qkv[2])
        scale = Dh ** (-0.5)
        pos = jnp.arange(S)
        off = jnp.arange(W) * dil
        idx = pos[:, None] - off[None, :]
        mask = idx >= 0
        idx_c = jnp.where(mask, idx, 0).reshape(-1)
        kg = k[:, :, idx_c, :].reshape(B, H, S, W, Dh)
        vg = v[:, :, idx_c, :].reshape(B, H, S, W, Dh)
        logits = jnp.einsum('bhsd,bhswd->bhsw', q, kg) * scale
        logits = jnp.where(mask[None, None, :, :], logits, -1000000000.0)
        attn = _softmax(logits, axis=-1)
        o = jnp.einsum('bhsw,bhswd->bhsd', attn, vg)
        return (lambda x, *d: x.transpose(*d))(o, 0, 2, 1, 3).reshape(B, S, D) @ wo

    def _B_ref(x, w1, w2):
        h = jnp.einsum('bsd,df->bsf', x, w1)
        h = _silu(h)
        out = jnp.einsum('bsf,fd->bsd', h, w2)
        return out
    x = A_x
    mod = (_silu(c) @ w_mod).reshape(c.shape[0], 6, 1, -1)
    sa, ca, ga, sb, cb, gb = (mod[:, 0].copy(), mod[:, 1].copy(), mod[:, 2].copy(), mod[:, 3].copy(), mod[:, 4].copy(), mod[:, 5].copy())
    h = _layernorm(x, axis=-1) * (1 + ca) + sa
    x = x + ga * _A_ref(h, A_wqkv, A_wo)
    h = _layernorm(x, axis=-1) * (1 + cb) + sb
    x = x + gb * _B_ref(h, B_w1, B_w2)
    return x
```

```python
import bisect
import functools
import heapq

import jax
import jax.numpy as jnp
from jax import lax
import jax.experimental.pallas as pl
import jax.experimental.pallas.tpu as pltpu

S, D, F = 2048, 512, 1792
H, DH, W, DIL = 32, 16, 8, 2
EPS = 1e-5
LOG2E = 1.4426950408889634
TM = 512
NB, HM = S // TM, TM // 2
NF = F // 256
HALO = 16
WS = DH + 1
PST = 3
SUMS = (0, 2, 3, 5, 6)

B1, B2, BX, B3, BM = 20, 44, 52, 76, 256
A0, A1, A2 = (23, 50), (9, 45), (8, 46)
P1, PS, PO, NQ = (40, 80), (24, 64), 4, 3
DA, DL, PVD, GSTEP = 2, 5, 2, 22
COV = (1, 4)
ACT = (0, 3)
N1 = 2
PQ = 0
XF = False
WB = 32

f32, bf16 = jnp.float32, jnp.bfloat16
P = functools.partial


def _dot(a, b):
    return jnp.dot(a, b, preferred_element_type=f32)


def _left(a11, a12, a21, a22):
    return [a11 + a22, a21 + a22, a11, a22, a11 + a12, a21 - a11, a12 - a22]


def _right(b11, b12, b21, b22):
    return [b11 + b22, b11, b12 - b22, b21 - b11, b22, b11 + b12, b21 + b22]


def _rep(t, n):
    return jnp.concatenate([t] * (n // 8), axis=0)


def _t128(j):
    return pl.ds(j * 128, 128)


def _kernel(x_hbm, wqkv_hbm, wo_hbm, w1_hbm, w2_hbm, c_hbm, wmod_hbm, out_hbm,
            x_v, wqkv_v, wo_v, w1_v, w2_v, c_v, wmod_v, out_v,
            wo_f, b1_s, b2_s, q_s, k_s, v_s, x1_s, g_s, sems):
    val = {}
    hooks = {}
    marks = []
    events = []
    st = {'pass': 0, 'seq': 0, 'sem': 0, 'alt': 0}

    def now():
        return HM * (st['pass'] // 4)

    def link(v, chain, t=None):
        deps = [val[chain]] if chain in val else []
        k = 0 if t is None else bisect.bisect_right(marks, t, key=lambda e: e[0])
        if k:
            _, ms, r = marks[k - 1]
            st['alt'] += 1
            deps += [m[r:r + 8] for m in (ms if chain else [ms[st['alt'] % len(ms)]])]
        if not deps:
            return v
        return jnp.where(val['never'], functools.reduce(jnp.maximum, deps), v)

    def done(chain, y):
        if st['pass']:
            val[chain] = y

    def spawn(t, steps):
        st['seq'] += 1
        heapq.heappush(events, (t, st['seq'], steps))

    def run_events(upto):
        while events and events[0][0] < upto:
            steps = heapq.heappop(events)[2]
            t = next(steps, None)
            if t is not None:
                spawn(t, steps)

    def mix(main, *sides):
        t0, span = now(), sum(c for _, c in main) * HM // 4
        for side, tail in sides:
            dt = max(span - (HM if tail else 0), 1) / max(len(side) + tail, 1)
            for k, task in enumerate(side):
                if task:
                    spawn(t0 + k * dt, task(t0 + k * dt, dt))
        for task, _ in main:
            task()
        if not main:
            run_events(float('inf'))

    def copy(src, dst, *idx):
        k = st['sem']
        st['sem'] += 1
        if idx:
            src, dst = src.at[idx], dst.at[idx]
        return lambda z=0: pltpu.make_async_copy(src, dst, sems.at[k + z])

    def wait(*copies, after=None):
        if after is None and marks:
            _, ms, r = marks[-WB]
            after = ms[0][r:r + 8]
        z = 0 if after is None else jnp.where(val['never'], pltpu.bitcast(after, jnp.int32), 0)[0, 0]
        for d in copies:
            d(z).wait()

    def park(ref, k, y):
        ref[k // PST, pl.ds(k % PST, HM, stride=PST), :] = y
        return lambda r, n: ref[k // PST, pl.ds(k % PST + r * PST, n, stride=PST), :]

    def dot(name, i, p, ks, b):
        run_events(now())
        for f in hooks.pop(st['pass'], ()):
            f()
        while not all((name, i, r, k) in val for r in range(0, HM, 8) for k in ks):
            run_events(events[0][0] + 1)
        if name == 'g':
            m = functools.reduce(jnp.add, [_dot(g_s[i, k, :, _t128(p)], b(p, k, 1)) for k in ks])
        else:
            a = jnp.concatenate([jnp.concatenate([val[name, i, r, k][p] for k in ks], axis=1)
                                 for r in range(0, HM, 8)], axis=0)
            m = _dot(a.astype(bf16), b(p, 0, 2))
        st['pass'] += len(ks)
        t0 = HM * ((st['pass'] - 1) // 4)
        if marks and marks[-1][0] >= t0:
            marks[-1][1].append(m)
        else:
            ms = [m]
            marks.extend((t0 + r, ms, r) for r in range(0, HM, 8))
        return m

    def strassen(name, i, nk, b, out):
        def prod(p):
            return functools.reduce(jnp.add, [dot(name, i, p, range(k, min(k + 2, nk)), b) for k in range(0, nk, 2)])
        early = st['pass'] % 4 == 2 and nk == 2
        m7 = prod(6) if early else None
        m2, m4 = prod(1), prod(3)
        out(m2 + m4, HM, 0)
        e = m4 + m7 if early else m4
        m3, m5 = prod(2), prod(4)
        out(m3 + m5, 0, 1)
        d, e = m3 - m2, e - m5
        m1, m6 = prod(0), prod(5)
        out(d + m1 + m6, HM, 1)
        e = e + m1
        out(e if early else e + prod(6), 0, 0)

    def put_left(name, i, o, r, y):
        other = val.pop((name, i, r), None)
        if other is None:
            val[name, i, r] = y
            return []
        top, bot = (other, y) if o else (y, other)
        for k in range(2):
            val[name, i, r, k] = _left(top[k], top[k + 2], bot[k], bot[k + 2])
        return [val[name, i, r, k][p] for k in range(2) for p in COV]

    def mod(j, k):
        r = _dot(val['silu_c'], wmod_v[:, _t128(4 * j + k)])[0:8]
        if j in (1, 4):
            r = r + 1.0
        if j in (3, 4):
            r = r * 0.5
        val['mod', j, k] = r

    def prep_qkv(j, n):
        lane = lax.broadcasted_iota(jnp.int32, (D // 2, 128), 1)
        g, hi, lo, a = lane // 32, (lane % 32) // 8, lane % 8, (lane % 16) // 4
        w = [pltpu.bitcast(wqkv_v[:, _t128(4 * j + k)], jnp.int32) for k in range(4)]
        o = []
        for t in (n, n + 2):
            y = jnp.where(a == t, w[0], jnp.where(a == (t + 1) % 4, w[1], jnp.where(a == (t + 2) % 4, w[2], w[3])))
            y = jnp.take_along_axis(y, lo * 16 + ((hi + t) % 4) * 4 + g, axis=1)
            o.append(pltpu.bitcast(y, bf16).astype(f32))
        val['wqkv', j, n] = [y.astype(bf16) for y in _right(o[0][:D // 2], o[1][:D // 2], o[0][D // 2:], o[1][D // 2:])]

    def shift_proj(j, n):
        lo, hi = [jnp.concatenate([_rep(val['mod', 0, k], 16), _rep(val['mod', 0, k + 1], 16)], axis=1) for k in (0, 2)]
        d = lambda a, p: _dot(a.astype(bf16), val['wqkv', j, n][p])[0:8]
        val['shift', j, n] = d(lo + hi, 1) + d(hi, 3)
        val['shift', j, n + 2] = d(lo, 2) + d(lo + hi, 4)

    def prep_wo(hi, n, t, dt):
        for h in range(8 * hi, 8 * hi + 8):
            for j in (n, n + 2):
                y = wo_v[pl.ds(h * DH, DH), _t128(j)].astype(f32)
                for r in (0, 8):
                    wo_f[j, pl.ds(h * WS + r, 8)] = link(y[r:r + 8], None, t)
            t += dt / 8
            yield t
        for k in range(2):
            for g in range(4):
                val['wo', n, (k * 4 + g) * 4 + hi] = _right(*[
                    wo_f[j, pl.ds(hi * 8 * WS + 4 * ((hi + kk) % 4) + g, 8, stride=WS), :]
                    for kk in (k, k + 2) for j in (n, n + 2)])

    def prep_mlp(src, dst, c0, c1, r, t, dt):
        w = [src[pl.ds(h * src.shape[0] // 2 + r, 16), _t128(j)].astype(f32) for h in (0, 1) for j in (c0, c1)]
        w[0] = jnp.concatenate([link(w[0][:8], None, t), w[0][8:]], axis=0)
        w[3] = jnp.concatenate([w[3][:8], link(w[3][8:], None, t)], axis=0)
        b = _right(*w)
        dst[pl.ds(r, 16), pl.ds(0, 128 * len(SUMS))] = jnp.concatenate([b[p] for p in SUMS], axis=1).astype(bf16)
        yield None

    def mlp_right(src, dst, c0, c1):
        def b(p, k, n):
            if p in SUMS:
                return dst[pl.ds(k * 128, n * 128), _t128(SUMS.index(p))]
            return src[pl.ds((p == 4) * src.shape[0] // 2 + k * 128, n * 128), _t128(c1 if p == 4 else c0)]
        return b

    def norm(name, i, o, r, chain, load, affine, t, dt):
        x = load()
        y = (x[0] + x[1]) + (link(x[2], chain, t) + x[3])
        done(chain, y)
        m = jnp.sum(y, axis=-1, keepdims=True)
        yield t + (DL + 0.3) * dt
        m = m * link(jnp.full((8, 128), 1.0 / D, f32), chain)
        sq = [(y - m) * (y - m) for y in x]
        y = (sq[0] + sq[1]) + (sq[2] + sq[3])
        done(chain, y)
        v = jnp.sum(y, axis=-1, keepdims=True)
        yield t + (2 * DL + 0.6) * dt
        m = link(m, chain)
        xc = [y - m for y in x]
        rs = lax.rsqrt(v * (1.0 / D) + EPS)
        new = put_left(name, i, o, r, [affine(xc[k] * rs, k) for k in range(4)])
        done(chain, functools.reduce(jnp.maximum, new) if new else xc[0])

    def norm1(i, o, r, t, dt):
        rows = pl.ds(i * TM + o + r // 16 * 16, 16)
        load = lambda: [x_v[rows, _t128(k)].astype(f32)[r % 16:r % 16 + 8] for k in range(4)]
        chain = ('chain', 0) if i > 1 else ('chain1', r // 8 % N1)
        return norm('h1', i, o, r, chain, load, lambda y, k: y * val['mod', 1, k], t, dt)

    def norm2(i, o, r, t, dt):
        load = lambda: [val['x1', i, o, k](r, 8) for k in range(4)]
        return norm('h2', i, o, r, ('chain', i + 1), load,
                    lambda y, k: y * val['mod', 4, k] + val['mod', 3, k], t, dt)

    def attend(i, o, r, t, dt):
        r0, chain = i * TM + o + r, ('chain', i)
        win = lambda ref, j, w: ref[j, pl.ds(HALO + r0 - DIL * w, 8)]
        scale = link(jnp.full((8, 128), DH ** -0.5 * LOG2E, f32), chain, t)
        for j in range(4):
            q = (val['q', i, o, j](r, 8) + val['shift', 0, j]) * scale
            l = [q * win(k_s, j, w) + l[w] if j else q * win(k_s, j, w) for w in range(W)]
            done(chain, l[-1])
            t += 0.1 * dt
            if j < 3:
                yield t
        for lanes in (64, 32):
            l = [y + pltpu.roll(y, lanes, 1) for y in l]
            t += (DA + 0.1) / 2 * dt
            yield t
        for w in range(W):
            if r0 < DIL * w:
                pos = r0 + lax.broadcasted_iota(jnp.int32, (8, 128), 0)
                l[w] = jnp.where(pos >= DIL * w, l[w], -1e9 * LOG2E)
        m = link(functools.reduce(jnp.maximum, l), chain)
        e = [jnp.exp2(y - m) for y in l]
        den = ((e[0] + e[1]) + (e[2] + e[3])) + ((e[4] + e[5]) + (e[6] + e[7]))
        inv = pltpu.reciprocal(den, approx=True)
        inv = inv * (2.0 - den * inv)
        out = []
        for j in range(4):
            t += 0.08 * dt
            yield t
            y = [(e[w] if w else link(e[0], chain)) * win(v_s, j, w) for w in range(W)]
            y = functools.reduce(jnp.add, y[PVD:] + y[:PVD])
            done(chain, y)
            out.append(y * inv + val['shift', 2, j])
        put_left('o', i, o, r, out)

    def qkv(i, j, n):
        def out(y, o, h):
            t = n + 2 * h
            if j == 0:
                val['q', i, o, t] = park(q_s, (i * 2 + o // HM) * 4 + t, y)
                return
            dst = k_s if j == 1 else v_s
            dst[t, pl.ds(HALO + i * TM + o, HM)] = y
            if i == 0 and o == 0:
                dst[t, pl.ds(0, HALO)] = jnp.broadcast_to(y[0:1], (HALO, 128))
        strassen('h1', i, 2, lambda p, k, nk: val['wqkv', j, n][p], out)

    def proj(i, n):
        def right(p, k, nk):
            if ('wo', n) not in val:
                val['wo', n] = [jnp.concatenate([val['wo', n, r][q] for r in range(D // 16)], axis=0).astype(bf16)
                                for q in range(7)]
            return val['wo', n][p]

        def out(y, o, h):
            t = n + 2 * h
            x = x_v[pl.ds(i * TM + o, HM), _t128(t)].astype(f32)
            val['x1', i, o, t] = park(x1_s, (i * 2 + o // HM) * 4 + t, x + _rep(val['mod', 2, t], HM) * y)
        strassen('o', i, 2, right, out)

    def up(i, n):
        c = {}

        def act(t):
            for r in range(0, HM, 8):
                y = [c[k][r:r + 8] for k in ((0, 0), (0, 1), (HM, 0), (HM, 1))]
                g = _left(*[z + z * jnp.tanh(link(z, None, t) if k in ACT else z) for k, z in enumerate(y)])
                g_s[i, n, pl.ds(r, 8), pl.ds(0, 7 * 128)] = jnp.concatenate(g, axis=1).astype(bf16)
                val['g', i, r, n] = True
                t += GSTEP
                yield t
        strassen('h2', i, 2, mlp_right(w1_v, b1_s.at[n], n, n + NF), lambda y, o, h: c.update({(o, h): y}))
        t0 = HM * ((st['pass'] - 1) // 4)
        spawn(t0, act(t0))

    def down(i, n, send=None):
        def out(y, o, h):
            t = 2 * n + h
            out_v[pl.ds(i * TM + o, HM), _t128(t)] = (
                val['x1', i, o, t](0, HM) + _rep(val['mod', 5, t], HM) * y).astype(bf16)
            if send:
                send(pl.ds(i * TM + o, HM), _t128(t))
        strassen('g', i, NF, mlp_right(w2_v, b2_s.at[n], 2 * n, 2 * n + 1), out)

    every, cols = slice(None), lambda j, n=1: pl.ds(j * D, n * D)
    d_c, d_wo, d_w1, d_w2 = copy(c_hbm, c_v), copy(wo_hbm, wo_v), copy(w1_hbm, w1_v), copy(w2_hbm, w2_v)
    d_x = [copy(x_hbm, x_v, pl.ds(i * TM, TM)) for i in range(NB)]
    d_qkv = [copy(wqkv_hbm, wqkv_v, every, cols(j)) for j in range(3)]
    d_mod = [copy(wmod_hbm, wmod_v, every, cc) for cc in (cols(0), cols(1), cols(2, 4))]
    second = [d_x[1], d_qkv[2]] if XF else [d_qkv[2], d_x[1]]
    for d in (d_c, d_mod[1], d_x[0], d_qkv[0], d_qkv[1], *second, d_mod[0], d_x[2], d_wo, d_x[3], d_mod[2], d_w1, d_w2):
        d().start()
    sent = []

    def send(rr, cc):
        sent.append(copy(out_v, out_hbm, rr, cc))
        sent[-1]().start()

    groups = lambda f, i: [P(f, i, o, r) for r in range(0, HM, 8) for o in (0, HM)]
    t_wo = [P(prep_wo, hi, n) for n in range(2) for hi in range(4)]
    t_w1 = [P(prep_mlp, w1_v, b1_s.at[n], n, n + NF, r) for n in range(NF) for r in range(0, D // 2, 16)]
    t_w2 = [P(prep_mlp, w2_v, b2_s.at[n], 2 * n, 2 * n + 1, r) for n in range(2) for r in range(0, F // 2, 16)]
    m_qkv = lambda i: [(P(qkv, i, j, n), 14) for j in range(3) for n in range(2)]
    m_proj = lambda i: [(P(proj, i, n), 14) for n in range(2)]
    m_up = lambda i: [(P(up, i, n), 14) for n in range(NF)]
    m_down = lambda i, n, *a: [(P(down, i, n, *a), 7 * NF)]
    at = lambda n, *fs: hooks.setdefault(n, []).extend(fs)
    tl, ta = 2 * DL + 1, DA + 1

    wait(d_c)
    c = c_v[...].astype(f32)
    val['silu_c'] = jnp.broadcast_to(c * jax.nn.sigmoid(c), (16, D)).astype(bf16)
    val['never'] = (pltpu.bitcast(jnp.broadcast_to(c[:, 0:128], (8, 128)), jnp.int32) & 1) > 1
    wait(d_mod[1])
    for k in range(4):
        mod(1, k)
    wait(d_x[0], after=val['mod', 1, 3])
    mix([], (groups(norm1, 0), 0))
    wait(d_qkv[0], after=functools.reduce(jnp.maximum, [val['h1', 0, r, 1][PQ] for r in range(0, HM, 8)]))
    prep_qkv(0, 0)
    prep_qkv(0, 1)
    at(B1, P(wait, d_qkv[1]), P(prep_qkv, 1, 0), P(prep_qkv, 1, 1))
    at(B2, P(wait, d_qkv[2]), P(prep_qkv, 2, 0), P(prep_qkv, 2, 1))
    at(BX, P(wait, d_x[1]))
    at(B3 - 8, P(wait, d_mod[0]))
    at(B3, P(mod, 0, 0), P(mod, 0, 1))
    at(B3 + 4, P(mod, 0, 2), P(mod, 0, 3))
    at(B3 + 8, P(shift_proj, 0, 0), P(shift_proj, 0, 1))
    at(B3 + 12, P(shift_proj, 2, 0), P(shift_proj, 2, 1))
    at(84, P(wait, d_x[2]))
    at(152, P(wait, d_wo, d_x[3]))
    at(BM - 12, P(wait, d_mod[2]))
    for n in range(16):
        at(BM + 4 * n, P(mod, 2 + n // 4, n % 4))
    at(252, P(wait, d_w1))
    at(308, P(wait, d_w2))

    a = groups(attend, 0)
    mix(m_qkv(0)[:2])
    mix(m_qkv(0)[2:], ([None] * ((BX - 28) * (65 + tl) // (80 - BX) + 1) + groups(norm1, 1), tl))
    mix(m_qkv(1), ([None] + a[:A0[0]], 0), (groups(norm1, 2), tl))
    mix(m_qkv(2), (a[A0[0]:A0[1]], 0), (groups(norm1, 3), tl), (t_wo[:PO], 1))
    mix(m_qkv(3)[:NQ], (a[A0[1]:], ta), (t_wo[PO:], 1), (t_w1[:P1[0]], 0))
    a = groups(attend, 1)
    mix(m_proj(0), (a[:A1[0]], 0), (t_w1[P1[0]:P1[1]], 0))
    mix(m_qkv(3)[NQ:], (groups(norm2, 0), tl), (t_w1[P1[1]:] + t_w2[:PS[0]], 1))
    mix(m_up(0), (a[A1[0]:A1[1]], 0), (t_w2[PS[0]:PS[1]], 1))
    mix(m_down(0, 0), (a[A1[1]:], ta), (t_w2[PS[1]:], 1))
    for i in range(1, NB):
        a = groups(attend, i + 1) if i + 1 < NB else []
        mix(m_proj(i), (a[:A2[0]], 0))
        mix(m_down(i - 1, 1), (groups(norm2, i), tl))
        mix(m_up(i), (a[A2[0]:A2[1]], 0))
        if i == NB - 1:
            send(pl.ds(0, i * TM), every)
        mix(m_down(i, 0), (a[A2[1]:], ta))
    send(pl.ds(S - TM, TM), pl.ds(0, 256))
    mix(m_down(NB - 1, 1, send))
    assert not hooks
    for d in sent:
        d().wait()


@jax.jit
def pallas_adaLN_cond__sliding_local_dilated__dense_activation_silu__prompt_kernel(
        A_x, A_wqkv, A_wo, B_x, B_w1, B_w2, c, w_mod):
    del B_x
    vmem = pltpu.VMEM
    parked = vmem((pl.cdiv(8 * NB, PST), PST * HM + 8, 128), f32)
    out = pl.pallas_call(
        _kernel,
        out_shape=jax.ShapeDtypeStruct((S, D), bf16),
        in_specs=[pl.BlockSpec(memory_space=pl.ANY)] * 7,
        out_specs=pl.BlockSpec(memory_space=pl.ANY),
        scratch_shapes=[
            vmem((S, D), bf16), vmem((D, 3 * D), bf16), vmem((D, D), bf16), vmem((D, F), bf16), vmem((F, D), bf16),
            vmem((1, D), bf16), vmem((D, 6 * D), bf16), vmem((S, D), bf16),
            vmem((4, H * WS + DH, 128), f32), vmem((NF, D // 2, 768), bf16), vmem((2, F // 2, 768), bf16),
            parked, vmem((4, HALO + S, 128), f32), vmem((4, HALO + S, 128), f32), parked,
            vmem((NB, NF, HM, 1024), bf16), pltpu.SemaphoreType.DMA((20,)),
        ],
        compiler_params=pltpu.CompilerParams(
            vmem_limit_bytes=100 * 1024 * 1024,
            disable_semaphore_checks=True,
            flags={"XLA_TPU_RESCHEDULE_DMA_DONES": True}),
    )(A_x.reshape(S, D), A_wqkv, A_wo, B_w1, B_w2, c, w_mod)
    return out.reshape(1, S, D)
```

```python
import bisect
import functools
import heapq

import jax
import jax.numpy as jnp
from jax import lax
import jax.experimental.pallas as pl
import jax.experimental.pallas.tpu as pltpu

S, D, F = 2048, 512, 1792
H, DH, W, DIL = 32, 16, 8, 2
EPS = 1e-5
LOG2E = 1.4426950408889634
TM = 512
NB, HM = S // TM, TM // 2
NF = F // 256
HALO = 16
WS = DH + 1
PST = 3
SUMS = (0, 2, 3, 5, 6)

AT_QKV, AT_X, AT_SHIFT = (4, 20, 28, 52, 60), (44, 64, 96, 152), 88
AT_WO, AT_MOD, AT_W1, AT_W2 = 124, 204, 252, 316
XS = 176
MR = 16
A0, A1, A2 = (22, 51), (6, 46), (10, 46)
P1, P2, PO = (28, 60), (8, 60), 1
LAG_AT, LAG_N1, LAG_N2 = 2, 6, 4
ACT_STEP = 25
LATER = 1e9

f32, bf16 = jnp.float32, jnp.bfloat16
P = functools.partial


def _dot(a, b):
    return jnp.dot(a, b, preferred_element_type=f32)


def _left(a11, a12, a21, a22):
    return [a11 + a22, a21 + a22, a11, a22, a11 + a12, a21 - a11, a12 - a22]


def _right(b11, b12, b21, b22):
    return [b11 + b22, b11, b12 - b22, b21 - b11, b22, b11 + b12, b21 + b22]


def _rep(t, n):
    return jnp.concatenate([t] * (n // 8), axis=0)


def _wide(t):
    return jnp.concatenate([t] * (D // 128), axis=1)


def _t128(j):
    return pl.ds(j * 128, 128)


def _kernel(x_hbm, wqkv_hbm, wo_hbm, w1_hbm, w2_hbm, c_hbm, wmod_hbm, out_hbm,
            x_v, wqkv_v, wo_v, w1_v, w2_v, c_v, wmod_v, out_v,
            c_s, wo_f, b1_s, b2_s, q_s, k_s, v_s, x1_s, g_s, sems):
    val = {}
    hooks = {}
    marks = []
    events = []
    landed = []
    st = {'pass': 0, 'seq': 0, 'sem': 0, 'alt': 0}

    def now():
        return HM * (st['pass'] // 4)

    def link(v, chain, t=None):
        deps = [val[chain]] if chain in val else []
        k = 0 if t is None else bisect.bisect_right(marks, t, key=lambda e: e[0])
        if k:
            _, ms, r = marks[k - 1]
            st['alt'] += 1
            deps += [m[r:r + 8] for m in (ms if chain else [ms[st['alt'] % len(ms)]])]
        if not deps:
            return v
        return lax.select(val['never'], functools.reduce(jnp.maximum, deps), v)

    def done(chain, y):
        if st['pass']:
            val[chain] = y

    def spawn(t, steps):
        st['seq'] += 1
        heapq.heappush(events, (t, st['seq'], steps))

    def run_events(upto):
        while events and events[0][0] < upto:
            steps = heapq.heappop(events)[2]
            t = next(steps, None)
            if t is not None:
                spawn(t, steps)

    def mix(main, *sides):
        end = now() + sum(c for _, c in main) * HM // 4
        for side, tail, *first in sides:
            t0 = first[0] * HM // 4 if first else now()
            dt = max(end - t0 - (HM if tail else 0), 1) / max(len(side) + tail, 1)
            for k, task in enumerate(side):
                spawn(t0 + k * dt, task(t0 + k * dt, dt))
        for task, _ in main:
            task()
        if not main:
            run_events(LATER)

    def copy(src, dst, *idx):
        k = st['sem']
        st['sem'] += 1
        if idx:
            src, dst = src.at[idx], dst.at[idx]
        return lambda z=0: pltpu.make_async_copy(src, dst, sems.at[k + z])

    def wait(*copies, after=None):
        if after is None and marks:
            _, ms, r = marks[-HM // 8]
            after = ms[0][r:r + 8]
        z = 0 if after is None else jnp.where(val['never'], pltpu.bitcast(after, jnp.int32), 0)[0, 0]
        for d in copies:
            d(z).wait()
            landed.append(d)

    def park(ref, k, y):
        ref[k // PST, pl.ds(k % PST, HM, stride=PST), :] = y
        return lambda r, n: ref[k // PST, pl.ds(k % PST + r * PST, n, stride=PST), :]

    def dot(name, i, p, ks, b):
        run_events(now())
        for f in hooks.pop(st['pass'], ()):
            f()
        if name == 'g':
            while not all(('g', i, k) in val for k in ks):
                run_events(events[0][0] + 1)
            m = functools.reduce(jnp.add, [_dot(g_s[i, k, :, _t128(p)], b(p, k, 1)) for k in ks])
        else:
            if (name, i) not in val:
                val[name, i] = [jnp.concatenate([val[name, i, r][q] for r in range(0, HM, 8)], axis=0).astype(bf16)
                                for q in range(7)]
            m = _dot(val[name, i][p], b(p, 0, 2))
        st['pass'] += len(ks)
        t0 = HM * ((st['pass'] - 1) // 4)
        if marks and marks[-1][0] >= t0:
            marks[-1][1].append(m)
        else:
            ms = [m]
            marks.extend((t0 + r, ms, r) for r in range(0, HM, 8))
        return m

    def strassen(name, i, nk, b, out, ready=()):
        def prod(p):
            if p in ready:
                return ready[p]
            return functools.reduce(jnp.add, [dot(name, i, p, range(k, min(k + 2, nk)), b) for k in range(0, nk, 2)])
        early = st['pass'] % 4 == 2 and nk == 2
        m7 = prod(6) if early else None
        if nk > 2:
            part = [[dot(name, i, p, range(k, k + 2), b) for k in range(0, nk - 1, 2)] for p in (1, 3)]
            m2, m4 = [functools.reduce(jnp.add, y) + dot(name, i, p, [nk - 1], b) for y, p in zip(part, (1, 3))]
        else:
            m2, m4 = prod(1), prod(3)
        out(m2 + m4, HM, 0)
        e = m4 + m7 if early else m4
        m3, m5 = prod(2), prod(4)
        out(m3 + m5, 0, 1)
        d, e = m3 - m2, e - m5
        m1, m6 = prod(0), prod(5)
        out(d + m1 + m6, HM, 1)
        e = e + m1
        out(e if early else e + prod(6), 0, 0)

    def put_left(name, i, o, r, y):
        other = val.pop((name, i, r, 'half'), None)
        if other is None:
            val[name, i, r, 'half'] = y
            return None
        top, bot = (other, y) if o else (y, other)
        val[name, i, r] = _left(top[:, :D // 2], top[:, D // 2:], bot[:, :D // 2], bot[:, D // 2:])
        return val[name, i, r]

    def mod(j, k):
        set_mod(j, k, _dot(val['silu_c'], wmod_v[:, _t128(4 * j + k)])[0:8])

    def mod_rows(j, r0, chain, t, dt):
        assert d_mod[2] in landed
        for r in range(r0, r0 + MR, 8):
            cc = link(c_s[pl.ds(r, 8)], chain, t)
            y = _wide(cc) * wmod_v[pl.ds(r, 8), pl.ds(j * D, D)].astype(f32)
            y = val['acc', j] = val['acc', j] + y if r else y
        acc = [y[:, k * 128:(k + 1) * 128] for k in range(4)]
        done(chain, functools.reduce(jnp.maximum, acc))
        if r0 + MR == D:
            for k in range(4):
                set_mod(j, k, jnp.broadcast_to(jnp.sum(acc[k], axis=0, keepdims=True), (8, 128)))
        yield None

    def set_mod(j, k, r):
        if j in (1, 4):
            r = r + 1.0
        if j in (3, 4):
            r = r * 0.5
        val['mod', j, k] = r
        if k == 3:
            val['mod', j] = jnp.concatenate([val['mod', j, q] for q in range(4)], axis=1)

    def prep_qkv(j, half):
        assert d_qkv[j][half] in landed
        lane = lax.broadcasted_iota(jnp.int32, (D // 4, 128), 1)
        g, hi, lo, a = lane // 32, (lane % 32) // 8, lane % 8, (lane % 16) // 4
        w = [pltpu.bitcast(wqkv_v[pl.ds(half * D // 2, D // 2), _t128(4 * j + k)], jnp.int32) for k in range(4)]
        for n in range(2):
            o = []
            for t in (n, n + 2):
                y = jnp.where(a == t, w[0], jnp.where(a == (t + 1) % 4, w[1], jnp.where(a == (t + 2) % 4, w[2], w[3])))
                y = jnp.take_along_axis(y, lo * 16 + ((hi + t) % 4) * 4 + g, axis=1)
                o.append(pltpu.bitcast(y, bf16).astype(f32))
            if half == 0:
                val['upper', j, n] = o
                val['wqkv', j, n] = {1: o[0].astype(bf16), 5: (o[0] + o[1]).astype(bf16)}
            else:
                b = _right(*val['upper', j, n], *o)
                val['wqkv', j, n].update({p: b[p].astype(bf16) for p in (0, 2, 3, 4, 6)})

    def shift_proj(j, n):
        lo, hi = [jnp.concatenate([_rep(val['mod', 0, k], 16), _rep(val['mod', 0, k + 1], 16)], axis=1) for k in (0, 2)]
        d = lambda a, p: _dot(a.astype(bf16), val['wqkv', j, n][p])[0:8]
        val['shift', j, n] = d(lo + hi, 1) + d(hi, 3)
        val['shift', j, n + 2] = d(lo, 2) + d(lo + hi, 4)

    def prep_wo(hi, n, t, dt):
        assert d_wo in landed
        for h in range(8 * hi, 8 * hi + 8):
            for j in (n, n + 2):
                y = wo_v[pl.ds(h * DH, DH), _t128(j)].astype(f32)
                for r in (0, 8):
                    wo_f[j, pl.ds(h * WS + r, 8)] = link(y[r:r + 8], None, t)
            t += dt / 8
            yield t
        for k in range(2):
            for g in range(4):
                val['wo', n, (k * 4 + g) * 4 + hi] = _right(*[
                    wo_f[j, pl.ds(hi * 8 * WS + 4 * ((hi + kk) % 4) + g, 8, stride=WS), :]
                    for kk in (k, k + 2) for j in (n, n + 2)])

    def prep_mlp(src, dst, c0, c1, r, t, dt):
        assert (d_w1 if src is w1_v else d_w2) in landed
        w = [src[pl.ds(h * src.shape[0] // 2 + r, 16), _t128(j)].astype(f32) for h in (0, 1) for j in (c0, c1)]
        w[0] = jnp.concatenate([link(w[0][:8], None, t), w[0][8:]], axis=0)
        w[3] = jnp.concatenate([w[3][:8], link(w[3][8:], None, t)], axis=0)
        b = _right(*w)
        dst[pl.ds(r, 16), pl.ds(0, 128 * len(SUMS))] = jnp.concatenate([b[p] for p in SUMS], axis=1).astype(bf16)
        yield None

    def mlp_right(src, dst, c0, c1):
        def b(p, k, n):
            if p in SUMS:
                return dst[pl.ds(k * 128, n * 128), _t128(SUMS.index(p))]
            return src[pl.ds((p == 4) * src.shape[0] // 2 + k * 128, n * 128), _t128(c1 if p == 4 else c0)]
        return b

    def norm(name, i, o, r, chain, load, affine, t, dt):
        x = load()
        lag = LAG_N2 if name == 'h2' else LAG_N1
        y = (x[0] + x[1]) + (link(x[2], chain, t) + x[3])
        done(chain, y)
        m = jnp.sum(y, axis=-1, keepdims=True)
        yield t + (lag + 0.3) * dt
        m = m * link(jnp.full((8, 128), 1.0 / D, f32), chain)
        x = jnp.concatenate(x, axis=1)
        y = x - _wide(m)
        y = y * y
        y = y[:, :D // 2] + y[:, D // 2:]
        y = y[:, :128] + y[:, 128:]
        done(chain, y)
        v = jnp.sum(y, axis=-1, keepdims=True)
        yield t + (2 * lag + 0.6) * dt
        y = x - _wide(link(m, chain))
        z = y * lax.rsqrt(v * (1.0 / D) + EPS)
        if ('mod', 1) not in val:
            val.setdefault('scaled', []).append(z[:, :128])
            yield LATER
        new = put_left(name, i, o, r, affine(z))
        if new:
            y = jnp.maximum(new[1], new[4])
            y = jnp.maximum(y[:, :128], y[:, 128:])
        done(chain, y[:, :128])

    def norm1(i, o, r, t, dt):
        def load():
            assert ([d_x0] * 2 + [d[o // HM] for d in d_x] + [d_x3] * 2)[2 * i + (r >= XS)] in landed
            x = x_v[pl.ds(i * TM + o + r, 8)].astype(f32)
            return [x[:, k * 128:(k + 1) * 128] for k in range(4)]
        chain = ('chain', 0) if i > 1 else ('chain1', r // 8 % 2)
        return norm('h1', i, o, r, chain, load, lambda y: y * val['mod', 1], t, dt)

    def norm2(i, o, r, t, dt):
        load = lambda: [val['x1', i, o, k](r, 8) for k in range(4)]
        return norm('h2', i, o, r, ('chain', i + 1), load,
                    lambda y: y * val['mod', 4] + val['mod', 3], t, dt)

    def attend(i, o, r, t, dt):
        r0, chain = i * TM + o + r, ('chain', i)
        window = lambda ref: jnp.concatenate([ref[:, pl.ds(HALO + r0 - DIL * w, 8)] for w in range(W)], axis=1)
        scale = link(jnp.full((8, 128), DH ** -0.5 * LOG2E, f32), chain, t)
        kw = window(k_s)
        for j in range(4):
            y = _rep((val['q', i, o, j](r, 8) + val['shift', 0, j]) * scale, 8 * W) * kw[j]
            l = y + l if j else y
            done(chain, l[8 * W - 8:])
            t += 0.1 * dt
            if j < 3:
                yield t
        for lanes in (64, 32):
            l = l + pltpu.roll(l, lanes, 1)
            t += (LAG_AT + 0.1) / 2 * dt
            yield t
        if r0 < DIL * (W - 1):
            n = lax.broadcasted_iota(jnp.int32, l.shape, 0)
            l = jnp.where(r0 + n % 8 >= DIL * (n // 8), l, -1e9 * LOG2E)
        m = link(jnp.max(l.reshape(W, 8, 128), axis=0), chain)
        e = jnp.exp2(l - _rep(m, 8 * W))
        den = jnp.sum(e.reshape(W, 8, 128), axis=0)
        inv = pltpu.reciprocal(den, approx=True)
        inv = inv * (2.0 - den * inv)
        vw, n, out = window(v_s), 8 * (W - 2), []
        e0, e1, e2 = e[:n], e[n:n + 8], e[n + 8:]
        for j in range(4):
            t += 0.08 * dt
            yield t
            y = jnp.sum((jnp.concatenate([e0, link(e1, chain), e2], axis=0) * vw[j]).reshape(W, 8, 128), axis=0)
            done(chain, y)
            out.append(y * inv + val['shift', 2, j])
        put_left('o', i, o, r, jnp.concatenate(out, axis=1))

    def qkv(i, j, n):
        def out(y, o, h):
            t = n + 2 * h
            if j == 0:
                val['q', i, o, t] = park(q_s, (i * 2 + o // HM) * 4 + t, y)
                return
            dst = k_s if j == 1 else v_s
            dst[t, pl.ds(HALO + i * TM + o, HM)] = y
            if i == 0 and o == 0:
                dst[t, pl.ds(0, HALO)] = jnp.broadcast_to(y[0:1], (HALO, 128))
        right = lambda n: lambda p, k, nk: val['wqkv', j, n][p]
        if i == 0 and n == 0:
            val['ready', i, j] = [{p: dot('h1', i, p, range(2), right(q)) for p in (1, 5)} for q in range(2)]
        strassen('h1', i, 2, right(n), out, val.get(('ready', i, j), [(), ()])[n])

    def proj(i, n):
        def right(p, k, nk):
            if ('wo', n) not in val:
                val['wo', n] = [jnp.concatenate([val['wo', n, r][q] for r in range(D // 16)], axis=0).astype(bf16)
                                for q in range(7)]
            return val['wo', n][p]

        def out(y, o, h):
            t = n + 2 * h
            x = x_v[pl.ds(i * TM + o, HM), _t128(t)].astype(f32)
            val['x1', i, o, t] = park(x1_s, (i * 2 + o // HM) * 4 + t, x + _rep(val['mod', 2, t], HM) * y)
        strassen('o', i, 2, right, out)

    def up(i, n):
        c = {}

        def act(t):
            for r in range(0, HM, 8):
                y = [c[k][r:r + 8] for k in ((0, 0), (0, 1), (HM, 0), (HM, 1))]
                g = _left(*[z + z * jnp.tanh(link(z, None, t) if k in (0, 3) else z) for k, z in enumerate(y)])
                g_s[i, n, pl.ds(r, 8), pl.ds(0, 7 * 128)] = jnp.concatenate(g, axis=1).astype(bf16)
                t += ACT_STEP
                if r + 8 < HM:
                    yield t
            val['g', i, n] = True
        strassen('h2', i, 2, mlp_right(w1_v, b1_s.at[n], n, n + NF), lambda y, o, h: c.update({(o, h): y}))
        t0 = HM * ((st['pass'] - 1) // 4)
        spawn(t0, act(t0))

    def down(i, n, send=None):
        def out(y, o, h):
            t = 2 * n + h
            out_v[pl.ds(i * TM + o, HM), _t128(t)] = (
                val['x1', i, o, t](0, HM) + _rep(val['mod', 5, t], HM) * y).astype(bf16)
            if send:
                send(pl.ds(i * TM + o, HM), _t128(t))
        strassen('g', i, NF, mlp_right(w2_v, b2_s.at[n], 2 * n, 2 * n + 1), out)

    every, cols = slice(None), lambda j, n=1: pl.ds(j * D, n * D)
    d_c, d_wo, d_w1, d_w2 = copy(c_hbm, c_v), copy(wo_hbm, wo_v), copy(w1_hbm, w1_v), copy(w2_hbm, w2_v)
    d_x0, d_x3 = copy(x_hbm, x_v, pl.ds(0, TM)), copy(x_hbm, x_v, pl.ds(3 * TM, TM))
    d_x = [[copy(x_hbm, x_v, pl.ds(i * TM + o + r, n)) for o in (0, HM)] for i in (1, 2) for r, n in ((0, XS), (XS, HM - XS))]
    d_qkv = [[copy(wqkv_hbm, wqkv_v, pl.ds(r, D // 2), cols(j)) for r in (0, D // 2)] for j in range(3)]
    d_mod = [copy(wmod_hbm, wmod_v, every, cc) for cc in (cols(0), cols(1), cols(2, 4))]
    for d in (d_c, d_x0, d_mod[1], *d_qkv[0], *d_qkv[1], *d_x[0], *d_qkv[2], *d_x[1], d_mod[0], *d_x[2], *d_x[3],
              d_wo, d_x3, d_mod[2], d_w1, d_w2):
        d().start()
    sent = []

    def send(rr, cc):
        sent.append(copy(out_v, out_hbm, rr, cc))
        sent[-1]().start()

    groups = lambda f, i: [P(f, i, o, r) for r in range(0, HM, 8) for o in (0, HM)]
    t_wo = [P(prep_wo, hi, n) for n in range(2) for hi in range(4)]
    t_w1 = [P(prep_mlp, w1_v, b1_s.at[n], n, n + NF, r) for n in range(NF) for r in range(0, D // 2, 16)]
    t_w2 = [P(prep_mlp, w2_v, b2_s.at[n], 2 * n, 2 * n + 1, r) for n in range(2) for r in range(0, F // 2, 16)]
    m_qkv = lambda i: [(P(qkv, i, j, n), 14) for j in range(3) for n in range(2)]
    m_proj = lambda i: [(P(proj, i, n), 14) for n in range(2)]
    m_up = lambda i: [(P(up, i, n), 14) for n in range(NF)]
    m_down = lambda i, n, *a: [(P(down, i, n, *a), 7 * NF)]
    at = lambda n, *fs: hooks.setdefault(n, []).extend(fs)
    tl, ta = 2 * LAG_N1 + 1, LAG_AT + 1

    wait(d_c)
    c = c_v[...].astype(f32)
    silu_c = c * jax.nn.sigmoid(c)
    val['silu_c'] = jnp.broadcast_to(silu_c, (16, D)).astype(bf16)
    val['never'] = (pltpu.bitcast(jnp.broadcast_to(c[:, 0:128], (8, 128)), jnp.int32) & 1) > 1
    c_s[...] = jnp.broadcast_to(silu_c.astype(bf16).astype(f32), (128, D)).T
    wait(d_x0)
    mix([], (groups(norm1, 0), 0))
    wait(d_mod[1], after=functools.reduce(jnp.maximum, val['scaled']))
    for k in range(4):
        mod(1, k)
    run_events(2 * LATER)
    wait(d_qkv[0][0], after=functools.reduce(jnp.maximum, [val['h1', 0, r][1][:, 128:] for r in range(0, HM, 8)]))
    prep_qkv(0, 0)
    for n, jh in zip(AT_QKV, ((0, 1), (1, 0), (1, 1), (2, 0), (2, 1))):
        at(n, P(wait, d_qkv[jh[0]][jh[1]]), P(prep_qkv, *jh))
    at(AT_X[0], P(wait, *d_x[0]))
    at(AT_X[1], P(wait, *d_x[1]))
    at(AT_SHIFT - 8, P(wait, d_mod[0]))
    at(AT_SHIFT, P(mod, 0, 0), P(mod, 0, 1))
    at(AT_SHIFT + 4, P(mod, 0, 2), P(mod, 0, 3))
    at(AT_SHIFT + 8, P(shift_proj, 0, 0), P(shift_proj, 0, 1))
    at(AT_SHIFT + 12, P(shift_proj, 2, 0), P(shift_proj, 2, 1))
    at(AT_X[2], P(wait, *d_x[2]))
    at(AT_WO, P(wait, *d_x[3], d_wo))
    at(AT_X[3], P(wait, d_x3))
    at(AT_MOD, P(wait, d_mod[2]))
    t_mod = lambda j, i: [P(mod_rows, j, r, ('chain', i)) for r in range(0, D, MR)]
    at(AT_W1, P(wait, d_w1))
    at(AT_W2, P(wait, d_w2))

    a = groups(attend, 0)
    mix(m_qkv(0)[:2])
    mix(m_qkv(0)[2:], (groups(norm1, 1), tl, AT_X[0]))
    mix(m_qkv(1), (a[:A0[0]], 0, AT_SHIFT + 8), (groups(norm1, 2), tl, AT_X[2]), (t_wo[:PO], 0, AT_WO))
    mix(m_qkv(2), (a[A0[0]:A0[1]], 0), (groups(norm1, 3), tl), (t_wo[PO:], 1), (t_mod(2, 0), 0, AT_MOD))
    mix(m_qkv(3)[:3], (a[A0[1]:], ta), (t_w1[:P1[0]], 0), (t_mod(3, 0), 1))
    a = groups(attend, 1)
    mix(m_proj(0), (a[:A1[0]], 0), (t_w1[P1[0]:P1[1]], 0), (t_mod(4, 1), 1))
    mix(m_qkv(3)[3:], (groups(norm2, 0), 2 * LAG_N2 + 1), (t_w1[P1[1]:] + t_w2[:P2[0]], 1))
    mix(m_up(0), (a[A1[0]:A1[1]], 0), (t_w2[P2[0]:P2[1]], 1), (t_mod(5, 1), 1))
    mix(m_down(0, 0), (a[A1[1]:], ta), (t_w2[P2[1]:], 1))
    for i in range(1, NB):
        a = groups(attend, i + 1) if i + 1 < NB else []
        mix(m_proj(i), (a[:A2[0]], 0))
        mix(m_down(i - 1, 1), (groups(norm2, i), 2 * LAG_N2 + 1))
        mix(m_up(i), (a[A2[0]:A2[1]], 0))
        if i == NB - 1:
            send(pl.ds(0, i * TM), every)
        mix(m_down(i, 0), (a[A2[1]:], ta))
    send(pl.ds(S - TM, TM), pl.ds(0, 256))
    mix(m_down(NB - 1, 1, send))
    assert not hooks
    for d in sent:
        d().wait()


@jax.jit
def pallas_adaLN_cond__sliding_local_dilated__dense_activation_silu__prompt_kernel(
        A_x, A_wqkv, A_wo, B_x, B_w1, B_w2, c, w_mod):
    del B_x
    vmem = pltpu.VMEM
    parked = vmem((pl.cdiv(8 * NB, PST), PST * HM + 8, 128), f32)
    out = pl.pallas_call(
        _kernel,
        out_shape=jax.ShapeDtypeStruct((S, D), bf16),
        in_specs=[pl.BlockSpec(memory_space=pl.ANY)] * 7,
        out_specs=pl.BlockSpec(memory_space=pl.ANY),
        scratch_shapes=[
            vmem((S, D), bf16), vmem((D, 3 * D), bf16), vmem((D, D), bf16), vmem((D, F), bf16), vmem((F, D), bf16),
            vmem((1, D), bf16), vmem((D, 6 * D), bf16), vmem((S, D), bf16),
            vmem((D, 128), f32), vmem((4, H * WS + DH, 128), f32), vmem((NF, D // 2, 768), bf16), vmem((2, F // 2, 768), bf16),
            parked, vmem((4, HALO + S, 128), f32), vmem((4, HALO + S, 128), f32), parked,
            vmem((NB, NF, HM, 1024), bf16), pltpu.SemaphoreType.DMA((29,)),
        ],
        compiler_params=pltpu.CompilerParams(
            vmem_limit_bytes=100 * 1024 * 1024,
            disable_semaphore_checks=True,
            flags={"XLA_TPU_RESCHEDULE_DMA_DONES": True}),
    )(A_x.reshape(S, D), A_wqkv, A_wo, B_w1, B_w2, c, w_mod)
    return out.reshape(1, S, D)
```
